```python
import jax
import jax.numpy as jnp

def _softmax(x, axis=-1):
    return jax.nn.softmax(x, axis=axis)
def _gelu(x):
    return jax.nn.gelu(x, approximate=True)
def _silu(x):
    return jax.nn.silu(x)
def _sigmoid(x):
    return jax.nn.sigmoid(x)
def _layernorm(x, axis=-1, eps=1e-5):
    m = jnp.mean(x, axis=axis, keepdims=True)
    v = jnp.var(x, axis=axis, keepdims=True)
    return (x - m) / jnp.sqrt(v + eps)
def _scatter_add(tgt, idx, src, axis=0):
    return tgt.at[idx].add(src)
def _segment_sum(src, seg, n):
    return jax.ops.segment_sum(src, seg, n)
class _Rng:
    def __init__(self, key):
        self._k = key
    def _next(self):
        self._k, sub = jax.random.split(self._k)
        return sub
    def normal(self, shape):
        return jax.random.normal(self._next(), shape, dtype=jnp.bfloat16)
    def randint(self, lo, hi, shape):
        return jax.random.randint(self._next(), shape, lo, hi, dtype=jnp.int32)
    def uniform(self, shape, lo=0.0, hi=1.0):
        return jax.random.uniform(self._next(), shape, jnp.bfloat16, lo, hi)
    def permutation(self, n):
        return jax.random.permutation(self._next(), n)


kernel_name = 'gated_mix__compressed_kv_cla__ssm_conv_s5__prompt'

def setup_inputs():
    _rng = _Rng(jax.random.key(int.from_bytes(__import__("os").urandom(4), "little")))
    _w = (lambda a: (lambda t: t.astype(jnp.bfloat16) if jnp.issubdtype(t.dtype, jnp.floating) else t)(jnp.asarray(a)))
    def _A_setup():
        B, H, Sq, Sk, D, M = 1, 16, 2048, 2048, 256, 448
        Dc = 4 * D
        return {
            "x": _w((lambda *s: _rng.normal(s) * 0.05)(B, Sq, M)),
            "c_kv": _w((lambda *s: _rng.normal(s) * 0.05)(B, Sk, Dc)),
            "w_q": _w((lambda *s: _rng.normal(s) * 0.05)(M, H, D) * (M ** -0.5)),
            "w_uk": _w((lambda *s: _rng.normal(s) * 0.05)(Dc, H, D) * (Dc ** -0.5)),
            "w_uv": _w((lambda *s: _rng.normal(s) * 0.05)(Dc, H, D) * (Dc ** -0.5)),
            "w_o": _w((lambda *s: _rng.normal(s) * 0.05)(H, D, M) * ((H * D) ** -0.5)),
        }
    _A_in = _A_setup()

    def _B_setup():
        B, S, D = 1, 2048, 448
        P = D
        Lambda_re = -0.5 * jnp.exp((lambda *s: _rng.normal(s) * 0.05)(P))
        Lambda_im = (lambda *s: _rng.normal(s) * 0.05)(P) * 1.0
        B_re = (lambda *s: _rng.normal(s) * 0.05)(P, D) * (D ** -0.5)
        B_im = (lambda *s: _rng.normal(s) * 0.05)(P, D) * (D ** -0.5)
        C_re = (lambda *s: _rng.normal(s) * 0.05)(D, P) * (P ** -0.5)
        C_im = (lambda *s: _rng.normal(s) * 0.05)(D, P) * (P ** -0.5)
        log_dt = (lambda *s: _rng.normal(s) * 0.05)(P) * 0.3 - 2.0
        Dskip = (lambda *s: _rng.normal(s) * 0.05)(D)
        return {
            "x": _w((lambda *s: _rng.normal(s) * 0.05)(B, S, D)),
            "Lambda_re": _w(Lambda_re),
            "Lambda_im": _w(Lambda_im),
            "B_re": _w(B_re),
            "B_im": _w(B_im),
            "C_re": _w(C_re),
            "C_im": _w(C_im),
            "log_dt": _w(log_dt),
            "Dskip": _w(Dskip),
        }
    _B_in = _B_setup()

    return {
        "A_x": _A_in["x"],
        "A_c_kv": _A_in["c_kv"],
        "A_w_q": _A_in["w_q"],
        "A_w_uk": _A_in["w_uk"],
        "A_w_uv": _A_in["w_uv"],
        "A_w_o": _A_in["w_o"],
        "B_x": _B_in["x"],
        "B_Lambda_re": _B_in["Lambda_re"],
        "B_Lambda_im": _B_in["Lambda_im"],
        "B_B_re": _B_in["B_re"],
        "B_B_im": _B_in["B_im"],
        "B_C_re": _B_in["C_re"],
        "B_C_im": _B_in["C_im"],
        "B_log_dt": _B_in["log_dt"],
        "B_Dskip": _B_in["Dskip"],
        "gate_w": _w((lambda *s: _rng.normal(s) * 0.05)(448)),
    }

def reference(A_x, A_c_kv, A_w_q, A_w_uk, A_w_uv, A_w_o, B_x, B_Lambda_re, B_Lambda_im, B_B_re, B_B_im, B_C_re, B_C_im, B_log_dt, B_Dskip, gate_w):
    def _A_ref(x, c_kv, w_q, w_uk, w_uv, w_o):
        B, Sq, M = x.shape[0], x.shape[1], x.shape[2]
        Sk = c_kv.shape[1]
        H, D = w_q.shape[1], w_q.shape[2]
        q = jnp.einsum("bqm,mhd->bhqd", x, w_q)
        k = jnp.einsum("bkc,chd->bhkd", c_kv, w_uk)
        v = jnp.einsum("bkc,chd->bhkd", c_kv, w_uv)
        scores = jnp.einsum("bhqd,bhkd->bhqk", q, k) * (D ** -0.5)
        off = Sk - Sq
        qi = jnp.arange(Sq)[:, None]
        kj = jnp.arange(Sk)[None, :]
        cmask = kj <= (qi + off)
        scores = jnp.where(cmask[None, None], scores, -1e9)
        p = _softmax(scores, axis=-1)
        ctx = jnp.einsum("bhqk,bhkd->bhqd", p, v)
        return jnp.einsum("bhqd,hdm->bqm", ctx, w_o)

    def _B_ref(x, Lambda_re, Lambda_im, B_re, B_im, C_re, C_im, log_dt, Dskip):
        Bsz, L, H = x.shape
        Lam = Lambda_re + 1j * Lambda_im
        Bmat = B_re + 1j * B_im
        Cmat = C_re + 1j * C_im
        dt = jnp.exp(log_dt)
        Lam_bar = jnp.exp(dt * Lam)
        B_bar = ((Lam_bar - 1.0) / Lam)[:, None] * Bmat
        Bu = jnp.einsum("bld,pd->blp", x + 0j, B_bar)
        h = jnp.zeros_like(Bu[:, 0, :])
        hs = []
        for t in range(L):
            h = Lam_bar[None, :] * h + Bu[:, t, :]
            hs.append(h)
        hseq = jnp.stack(hs, 1)
        y = 2.0 * jnp.einsum("blp,dp->bld", hseq, Cmat).real + x * Dskip[None, None, :]
        return y

    x = A_x
    g = _sigmoid((x * gate_w).sum(-1, keepdims=True))
    a = _A_ref(x, A_c_kv, A_w_q, A_w_uk, A_w_uv, A_w_o)
    b = _B_ref(x, B_Lambda_re, B_Lambda_im, B_B_re, B_B_im, B_C_re, B_C_im, B_log_dt, B_Dskip)
    return g * a + (1 - g) * b
```

```python
import functools
import jax
import jax.numpy as jnp
import numpy as np
from jax import lax
import jax.experimental.pallas as pl
import jax.experimental.pallas.tpu as pltpu

S = 2048
M = 448
H = 16
D = 256
DC = 1024
BQ = 256
TB = 256
OB = 256
LOG2E = 1.4426950408889634
F32 = jnp.float32
BF16 = jnp.bfloat16
NT = (((1,), (1,)), ((), ()))
TN = (((0,), (0,)), ((), ()))
TT = (((0,), (1,)), ((), ()))


def _dot(a, b, dn=(((1,), (0,)), ((), ()))):
    return lax.dot_general(a, b, dn, preferred_element_type=F32)


def _unpack(x, odd):
    sh = (16 * (1 - odd)).astype(jnp.uint32)
    x = (x << sh) & jnp.uint32(0xFFFF0000)
    return pltpu.bitcast(x, F32)


def _col(v):
    return jnp.broadcast_to(v, (128, M)).T


def _kernel(xt_hbm, c_hbm, wq_hbm, wk_hbm, wv_hbm, wo_hbm, lre_ref, lim_ref, bre_hbm, bim_hbm,
            cre_hbm, cim_hbm, ldt_ref, dsk_ref, gw_ref, o_hbm,
            xt_s, c_s, wq_buf, wk_buf, wv_buf, wo_s, bc_s, q_s, k_s, v_s, g_s, ctx_s, o_s,
            wsem, isem, osem):
    def wcopies(p, slot):
        return (
            pltpu.make_async_copy(wq_hbm.bitcast(jnp.uint32).at[:, p, :], wq_buf.at[slot], wsem.at[slot, 0]),
            pltpu.make_async_copy(wk_hbm.bitcast(jnp.uint32).at[:, p, :], wk_buf.at[slot], wsem.at[slot, 1]),
            pltpu.make_async_copy(wv_hbm.bitcast(jnp.uint32).at[:, p, :], wv_buf.at[slot], wsem.at[slot, 2]),
        )
    cp_x = pltpu.make_async_copy(xt_hbm, xt_s, isem.at[0])
    cp_bc = [pltpu.make_async_copy(r, bc_s.at[j], isem.at[1 + j])
             for j, r in enumerate((bre_hbm, bim_hbm, cre_hbm, cim_hbm))]
    cp_c = pltpu.make_async_copy(c_hbm, c_s, isem.at[5])
    cp_wo = pltpu.make_async_copy(wo_hbm, wo_s, isem.at[6])
    cp_x.start()
    for cp in cp_bc:
        cp.start()
    cp_c.start()
    for cp in wcopies(0, 0):
        cp.start()
    cp_wo.start()

    lre = lre_ref[...].astype(F32).reshape(1, M)
    lim = lim_ref[...].astype(F32).reshape(1, M)
    dt = jnp.exp(ldt_ref[...].astype(F32).reshape(1, M)).astype(BF16).astype(F32)
    ar = dt * lre
    ai = dt * lim
    sub = lax.broadcasted_iota(jnp.int32, (8, M), 0)
    kk = (sub + 1).astype(F32)
    mag = jnp.exp(kk * ar)
    pr = mag * jnp.cos(kk * ai)
    pi = mag * jnp.sin(kk * ai)
    l1r, l1i = pr[0:1], pi[0:1]
    den = lre * lre + lim * lim
    cfr = ((l1r - 1.0) * lre + l1i * lim) / den
    cfi = (l1i * lre - (l1r - 1.0) * lim) / den
    steps = []
    for d in (1, 2, 4):
        steps.append((d, jnp.where(sub >= d, pr[d - 1:d], 0.0), jnp.where(sub >= d, pi[d - 1:d], 0.0)))
    gw_c = _col(gw_ref[...].astype(F32).reshape(1, M))
    dsk_c = _col(dsk_ref[...].astype(F32).reshape(1, M))

    cp_x.wait()
    for cp in cp_bc:
        cp.wait()
    car_r = jnp.zeros((8, M), F32)
    car_i = jnp.zeros((8, M), F32)
    for t in range(S // TB):
        xt = xt_s[:, t * TB:(t + 1) * TB]
        ur = _dot(xt, bc_s[0], TT)
        ui = _dot(xt, bc_s[1], TT)
        hr = (ur * cfr - ui * cfi).reshape(TB // 8, 8, M)
        hi = (ur * cfi + ui * cfr).reshape(TB // 8, 8, M)
        for d, mr, mi in steps:
            sr = pltpu.roll(hr, d, 1)
            si = pltpu.roll(hi, d, 1)
            hr, hi = hr + (mr * sr - mi * si), hi + (mr * si + mi * sr)
        outr, outi = [], []
        for r in range(TB // 8):
            vr = hr[r] + (pr * car_r - pi * car_i)
            vi = hi[r] + (pr * car_i + pi * car_r)
            car_r = jnp.broadcast_to(vr[7:8], (8, M))
            car_i = jnp.broadcast_to(vi[7:8], (8, M))
            outr.append(vr)
            outi.append(vi)
        hr = jnp.concatenate(outr, axis=0).astype(BF16)
        hi = jnp.concatenate(outi, axis=0).astype(BF16)
        yt = _dot(bc_s[2], hr, NT) - _dot(bc_s[3], hi, NT)
        xf = xt.astype(F32)
        z = jnp.sum(xf * jnp.tile(gw_c, (1, TB // 128)), axis=0, keepdims=True)
        g = 1.0 / (1.0 + jnp.exp(-z))
        g_s[:, t * TB:(t + 1) * TB] = g
        o_s[:, t * TB:(t + 1) * TB] = (1.0 - g) * (2.0 * yt + xf * jnp.tile(dsk_c, (1, TB // 128)))

    cp_c.wait()

    def head(h, carry):
        hp = h // 2
        odd = h % 2

        @pl.when(odd == 0)
        def _():
            @pl.when(hp + 1 < H // 2)
            def _():
                for cp in wcopies(hp + 1, (hp + 1) % 2):
                    cp.start()
            for cp in wcopies(hp, hp % 2):
                cp.wait()

        slot = hp % 2
        wqt = (_unpack(wq_buf[slot], odd) * (LOG2E * D ** -0.5)).T.astype(BF16)
        wk = _unpack(wk_buf[slot], odd).astype(BF16)
        wvt = _unpack(wv_buf[slot], odd).T.astype(BF16)
        q_s[...] = _dot(wqt, xt_s[...]).astype(BF16)
        k_s[...] = _dot(c_s[...], wk).astype(BF16)
        v_s[...] = _dot(wvt, c_s[...], NT).astype(BF16)

        row = lax.broadcasted_iota(jnp.int32, (BQ, BQ), 0)
        col = lax.broadcasted_iota(jnp.int32, (BQ, BQ), 1)
        cm = row <= col
        for i in range(S // BQ):
            r0 = i * BQ
            q = q_s[:, r0:r0 + BQ]
            sd = _dot(k_s[r0:r0 + BQ, :], q)
            sd = jnp.where(cm, sd, -1e30)
            m = jnp.max(sd, axis=0, keepdims=True)
            if i > 0:
                so = _dot(k_s[0:r0, :], q)
                m = jnp.maximum(m, jnp.max(so, axis=0, keepdims=True))
            pd = jnp.exp2(sd - m)
            l = jnp.sum(pd, axis=0, keepdims=True)
            acc = _dot(v_s[:, r0:r0 + BQ], pd.astype(BF16))
            if i > 0:
                po = jnp.exp2(so - m)
                l = l + jnp.sum(po, axis=0, keepdims=True)
                acc = acc + _dot(v_s[:, 0:r0], po.astype(BF16))
            sc = g_s[:, r0:r0 + BQ] / l
            ctx_s[h, :, r0:r0 + BQ] = (acc * sc).astype(BF16)
        return carry

    lax.fori_loop(0, H, head, 0)

    cp_wo.wait()
    ocps = []
    for j in range(S // OB):
        acc = o_s[:, j * OB:(j + 1) * OB]
        for hh in range(H):
            acc = acc + _dot(wo_s[hh], ctx_s[hh, :, j * OB:(j + 1) * OB])
        o_s[:, j * OB:(j + 1) * OB] = acc
        cp = pltpu.make_async_copy(o_s.at[:, j * OB:(j + 1) * OB], o_hbm.at[:, j * OB:(j + 1) * OB], osem.at[j])
        cp.start()
        ocps.append(cp)
    for cp in ocps:
        cp.wait()


@jax.jit
def pallas_gated_mix__compressed_kv_cla__ssm_conv_s5__prompt_kernel(A_x, A_c_kv, A_w_q, A_w_uk, A_w_uv, A_w_o, B_x, B_Lambda_re, B_Lambda_im, B_B_re, B_B_im,
         B_C_re, B_C_im, B_log_dt, B_Dskip, gate_w):
    vec = pl.BlockSpec(memory_space=pltpu.VMEM)
    hbm = pl.BlockSpec(memory_space=pltpu.HBM)
    xt = jnp.transpose(A_x[0])
    wot = jnp.transpose(A_w_o, (0, 2, 1))
    out = pl.pallas_call(
        _kernel,
        in_specs=[hbm, hbm, hbm, hbm, hbm, hbm, vec, vec, hbm, hbm, hbm, hbm, vec, vec, vec],
        out_specs=hbm,
        out_shape=jax.ShapeDtypeStruct((M, S), F32),
        scratch_shapes=[
            pltpu.VMEM((M, S), BF16),
            pltpu.VMEM((S, DC), BF16),
            pltpu.VMEM((2, M, D), jnp.uint32),
            pltpu.VMEM((2, DC, D), jnp.uint32),
            pltpu.VMEM((2, DC, D), jnp.uint32),
            pltpu.VMEM((H, M, D), BF16),
            pltpu.VMEM((4, M, M), BF16),
            pltpu.VMEM((D, S), BF16),
            pltpu.VMEM((S, D), BF16),
            pltpu.VMEM((D, S), BF16),
            pltpu.VMEM((1, S), F32),
            pltpu.VMEM((H, D, S), BF16),
            pltpu.VMEM((M, S), F32),
            pltpu.SemaphoreType.DMA((2, 3)),
            pltpu.SemaphoreType.DMA((7,)),
            pltpu.SemaphoreType.DMA((S // OB,)),
        ],
        compiler_params=pltpu.CompilerParams(vmem_limit_bytes=100 * 2**20),
    )(xt, A_c_kv[0], A_w_q, A_w_uk, A_w_uv, wot, B_Lambda_re, B_Lambda_im, B_B_re, B_B_im,
      B_C_re, B_C_im, B_log_dt, B_Dskip, gate_w)
    return jnp.transpose(out)[None]
```

```python
import jax
import jax.numpy as jnp
from jax import lax
import jax.experimental.pallas as pl
import jax.experimental.pallas.tpu as pltpu

S = 2048
M = 448
H = 16
D = 256
DC = 1024
BQ = 256
HB = 128
VS = [6, 6, 6, 6, 6, 6, 6, 6, 8, 8]
LCH = 6
TB = 256
OB = 256
LOG2E = 1.4426950408889634
F32 = jnp.float32
BF16 = jnp.bfloat16
NT = (((1,), (1,)), ((), ()))


def _dot(a, b, dn=(((1,), (0,)), ((), ()))):
    return lax.dot_general(a, b, dn, preferred_element_type=F32)


def _unpack(x, odd):
    sh = (16 * (1 - odd)).astype(jnp.uint32)
    x = (x << sh) & jnp.uint32(0xFFFF0000)
    return pltpu.bitcast(x, F32)


def _col(v):
    return jnp.broadcast_to(v, (128, M)).T


def _kernel(xt_hbm, c_hbm, wq_hbm, wk_hbm, wv_hbm, wo_hbm, lre_ref, lim_ref, bre_hbm, bim_hbm,
            cre_hbm, cim_hbm, ldt_ref, dsk_ref, gw_ref, o_hbm,
            xt_s, c_s, wq_buf, wk_buf, wv_buf, wo_s, bc_s, q_s, k_s, v_s, g_s, ctx_s, o_s, wk_t, cc_s, u_s, pw_s,
            wsem, isem, osem):
    def wcopy(j, hd):
        src, buf = ((wq_hbm, wq_buf), (wk_hbm, wk_buf), (wv_hbm, wv_buf))[j]
        pair = jnp.minimum(hd // 2, H // 2 - 1)
        return pltpu.make_async_copy(src.bitcast(jnp.uint32).at[:, pair, :], buf.at[hd % 2], wsem.at[hd % 2, j])

    XH = 2 * TB
    cp_x0 = pltpu.make_async_copy(xt_hbm.at[:, 0:XH], xt_s.at[:, 0:XH], isem.at[0])
    cp_x1 = pltpu.make_async_copy(xt_hbm.at[:, XH:S], xt_s.at[:, XH:S], isem.at[7])
    cp_bc = [pltpu.make_async_copy(r, bc_s.at[j], isem.at[1 + j])
             for j, r in enumerate((bre_hbm, bim_hbm, cre_hbm, cim_hbm))]
    cp_c = pltpu.make_async_copy(c_hbm, c_s, isem.at[5])
    cp_wo = pltpu.make_async_copy(wo_hbm, wo_s, isem.at[6])
    first = [cp_x0, cp_bc[0], cp_bc[1]]
    second = [cp_bc[2], cp_bc[3], cp_x1]
    for cp in first:
        cp.start()

    def unpack_k(hd):
        wk_t[...] = _unpack(wk_buf[hd % 2], hd % 2).astype(BF16)

    lre = lre_ref[...].astype(F32).reshape(1, M)
    lim = lim_ref[...].astype(F32).reshape(1, M)
    dt = jnp.exp(ldt_ref[...].astype(F32).reshape(1, M)).astype(BF16).astype(F32)
    ar = dt * lre
    ai = dt * lim
    sub = lax.broadcasted_iota(jnp.int32, (8, M), 0)
    kk = (sub + 1).astype(F32)
    mag = jnp.exp(kk * ar)
    pr = mag * jnp.cos(kk * ai)
    pi = mag * jnp.sin(kk * ai)
    l1r, l1i = pr[0:1], pi[0:1]
    den = lre * lre + lim * lim
    cfr = ((l1r - 1.0) * lre + l1i * lim) / den
    cfi = (l1i * lre - (l1r - 1.0) * lim) / den
    steps = []
    for d in (1, 2, 4):
        steps.append((d, jnp.where(sub >= d, pr[d - 1:d], 0.0), jnp.where(sub >= d, pi[d - 1:d], 0.0)))
    pw_s[0] = pr
    pw_s[1] = pi
    for j, (_, mr, mi) in enumerate(steps):
        pw_s[2 + 2 * j] = mr
        pw_s[3 + 2 * j] = mi
    gw_c = _col(gw_ref[...].astype(F32).reshape(1, M))
    dsk_c = _col(dsk_ref[...].astype(F32).reshape(1, M))

    for cp in first:
        cp.wait()
    for cp in second:
        cp.start()
    h0 = jnp.int32(0)
    wcopy(1, h0).start()
    cp_c.start()
    wcopy(0, h0).start()
    wcopy(2, h0).start()

    MF = 384
    b3 = jnp.concatenate([bc_s[0, MF:M, :], bc_s[1, MF:M, :]], axis=0)

    def u_proj(t):
        xc = xt_s[:, t * TB:(t + 1) * TB].astype(F32).T.astype(BF16)
        u3 = _dot(xc, b3, NT)
        ur = jnp.concatenate([_dot(xc, bc_s[0, 0:MF, :], NT), u3[:, :M - MF]], axis=1)
        ui = jnp.concatenate([_dot(xc, bc_s[1, 0:MF, :], NT), u3[:, M - MF:]], axis=1)
        u_s[0, t * TB:(t + 1) * TB, :] = ur * cfr - ui * cfi
        u_s[1, t * TB:(t + 1) * TB, :] = ur * cfi + ui * cfr
        xf = xt_s[:, t * TB:(t + 1) * TB].astype(F32)
        z = jnp.sum(xf * jnp.tile(gw_c, (1, TB // 128)), axis=0, keepdims=True)
        g = 1.0 / (1.0 + jnp.exp(-z))
        g_s[:, t * TB:(t + 1) * TB] = g
        o_s[:, t * TB:(t + 1) * TB] = xf * jnp.tile(dsk_c, (1, TB // 128))

    def scan(t, car_r, car_i):
        pr, pi = pw_s[0], pw_s[1]
        steps = [(d, pw_s[2 + 2 * j], pw_s[3 + 2 * j]) for j, d in enumerate((1, 2, 4))]
        hr = u_s[0, t * TB:(t + 1) * TB, :].reshape(TB // 8, 8, M)
        hi = u_s[1, t * TB:(t + 1) * TB, :].reshape(TB // 8, 8, M)
        for d, mr, mi in steps:
            sr = pltpu.roll(hr, d, 1)
            si = pltpu.roll(hi, d, 1)
            hr, hi = hr + (mr * sr - mi * si), hi + (mr * si + mi * sr)
        outr, outi, cars = [], [], []
        for r in range(TB // 8):
            vr = hr[r] + (pr * car_r - pi * car_i)
            vi = hi[r] + (pr * car_i + pi * car_r)
            car_r = jnp.broadcast_to(vr[7:8], (8, M))
            car_i = jnp.broadcast_to(vi[7:8], (8, M))
            outr.append(vr)
            outi.append(vi)
            cars.append(vr)
        hr = jnp.concatenate(outr, axis=0)
        hi = jnp.concatenate(outi, axis=0)
        hh = jnp.concatenate([hr[:, :MF], hi[:, :MF], hr[:, MF:], hi[:, MF:]], axis=1).astype(BF16)
        return hh, car_r, car_i, cars

    nt = S // TB
    for t in range(nt):
        if t == 2:
            for cp in second:
                cp.wait()
        if t == nt - 2:
            wcopy(1, h0).wait()
            cp_c.wait()
            wcopy(1, h0 + 1).start()
            cp_wo.start()
            unpack_k(h0)
        u_proj(t)

    def head(h, carry):
        hn = h + 1
        wcopy(1, h + 2).start()
        wcopy(0, hn).start()
        wcopy(2, hn).start()
        wcopy(1, hn).wait()
        wcopy(0, h).wait()
        wcopy(2, h).wait()
        wqt = (_unpack(wq_buf[h % 2], h % 2) * (LOG2E * D ** -0.5)).T.astype(BF16)
        wvt = _unpack(wv_buf[h % 2], h % 2).T.astype(BF16)

        row = lax.broadcasted_iota(jnp.int32, (HB, HB), 0)
        col = lax.broadcasted_iota(jnp.int32, (HB, HB), 1)
        cm = row <= col
        nb = S // BQ

        def red8(x, op):
            parts = [x[r:r + 8] for r in range(0, x.shape[0], 8)]
            while len(parts) > 1:
                parts = [op(parts[j], parts[j + 1]) for j in range(0, len(parts), 2)]
            return parts[0]

        def s_chunk(i, c, m8):
            r0 = c * BQ
            if c == i:
                st = _dot(k_s[r0:r0 + HB, :], q_s[:, r0:r0 + BQ])
                sb = _dot(k_s[r0 + HB:r0 + BQ, :], q_s[:, r0 + HB:r0 + BQ])
                st = jnp.concatenate([jnp.where(cm, st[:, :HB], -1e30), st[:, HB:]], axis=1)
                sb = jnp.where(cm, sb, -1e30)
                mt = red8(st, jnp.maximum)
                mm = jnp.concatenate([mt[:, :HB], jnp.maximum(mt[:, HB:], red8(sb, jnp.maximum))], axis=1)
                s = (st, sb)
            else:
                s = _dot(k_s[r0:r0 + BQ, :], q_s[:, i * BQ:(i + 1) * BQ])
                mm = red8(s, jnp.maximum)
            return s, (mm if m8 is None else jnp.maximum(m8, mm))

        def e_chunk(s, mb, l8):
            if isinstance(s, tuple):
                pt = jnp.exp2(s[0] - jnp.tile(mb, (HB // 8, 1)))
                pb = jnp.exp2(s[1] - jnp.tile(mb[:, HB:], (HB // 8, 1)))
                lt = red8(pt, jnp.add)
                ll = jnp.concatenate([lt[:, :HB], lt[:, HB:] + red8(pb, jnp.add)], axis=1)
                p = (pt.astype(BF16), pb.astype(BF16))
            else:
                p = jnp.exp2(s - jnp.tile(mb, (BQ // 8, 1)))
                ll = red8(p, jnp.add)
                p = p.astype(BF16)
            return p, (ll if l8 is None else l8 + ll)

        def pv_chunk(c, p, acc):
            r0 = c * BQ
            if isinstance(p, tuple):
                r = _dot(v_s[:, r0:r0 + HB], p[0])
                rb = _dot(v_s[:, r0 + HB:r0 + BQ], p[1])
                r = jnp.concatenate([r[:, :HB], r[:, HB:] + rb], axis=1)
            else:
                r = _dot(v_s[:, r0:r0 + BQ], p)
            return r if acc is None else acc + r

        def fin(i, acc, l8):
            l = jnp.sum(l8, axis=0, keepdims=True)
            sc = g_s[:, i * BQ:(i + 1) * BQ] / l
            ctx_s[h, :, i * BQ:(i + 1) * BQ] = (acc * sc).astype(BF16)

        def vproj(j0, j1):
            v_s[:, j0 * BQ:j1 * BQ] = _dot(wvt, c_s[j0 * BQ:j1 * BQ, :], NT).astype(BF16)

        k_s[...] = _dot(c_s[...], wk_t[...]).astype(BF16)
        q_s[...] = _dot(wqt, xt_s[...]).astype(BF16)
        s0, m8 = s_chunk(0, 0, None)
        cur_s = [s0]
        vproj(0, VS[0])
        unpack_k(hn)
        prev = None
        for i in range(nb + 1):
            if i < nb:
                m = jnp.max(m8, axis=0, keepdims=True)
            if VS[i + 1] > VS[i]:
                vproj(VS[i], VS[i + 1])
            nxt_s, m8n, ps, l8, acc = [], None, [], None, None
            for c in range(i + 2):
                m8p = m8n
                if i + 1 < nb:
                    s, m8n = s_chunk(i + 1, c, m8n)
                    nxt_s.append(s)
                if i < nb and c <= i:
                    mb = jnp.broadcast_to(m, (8, BQ))
                    if l8 is not None and i < LCH:
                        mb = jnp.where(l8 < 0.0, 0.0, mb)
                    if m8p is not None and i < 6:
                        mb = jnp.where(m8p < -3.4e38, 0.0, mb)
                    p, l8 = e_chunk(cur_s[c], mb, l8)
                    ps.append(p)
                if prev is not None and c <= prev[0]:
                    acc = pv_chunk(c, prev[1][c], acc)
            if prev is not None:
                fin(prev[0], acc, prev[2])
            prev = (i, ps, l8)
            cur_s, m8 = nxt_s, m8n
        return carry

    lax.fori_loop(0, H, head, 0)

    wcopy(1, h0 + H + 1).wait()
    wcopy(0, h0 + H).wait()
    wcopy(2, h0 + H).wait()
    cp_wo.wait()
    ocps = []
    cre = 2.0 * bc_s[2].astype(F32)
    cim = -2.0 * bc_s[3].astype(F32)
    cc_s[...] = jnp.concatenate([cre[:, :MF], cim[:, :MF], cre[:, MF:], cim[:, MF:]], axis=1).astype(BF16)
    car_r = jnp.zeros((8, M), F32)
    car_i = jnp.zeros((8, M), F32)
    for j in range(S // OB):
        cols = slice(j * OB, (j + 1) * OB)
        st, car_r, car_i, cars = scan(j, car_r, car_i)
        acc = _dot(wo_s[0], ctx_s[0, :, cols])
        for hh in range(1, H):
            w = wo_s[hh]
            cr = jnp.abs(cars[min(3 * hh, TB // 8 - 1)])
            cr = jnp.minimum(jnp.minimum(cr[:, 0:128], cr[:, 128:256]), jnp.minimum(cr[:, 256:384], cr[:, 320:448]))
            tie = jnp.tile(cr, (2, D // 128)) < 0.0
            w = jnp.concatenate([jnp.where(tie, 0.0, w[:16].astype(F32)).astype(BF16), w[16:]], axis=0)
            acc = acc + _dot(w, ctx_s[hh, :, cols])
            if hh == 13:
                acc = acc + (1.0 - g_s[:, cols]) * (_dot(cc_s[...], st, NT) + o_s[:, cols])
        o_s[:, cols] = acc
        cp = pltpu.make_async_copy(o_s.at[:, j * OB:(j + 1) * OB], o_hbm.at[:, j * OB:(j + 1) * OB], osem.at[j])
        cp.start()
        ocps.append(cp)
    for cp in ocps:
        cp.wait()


@jax.jit
def pallas_gated_mix__compressed_kv_cla__ssm_conv_s5__prompt_kernel(A_x, A_c_kv, A_w_q, A_w_uk, A_w_uv, A_w_o, B_x, B_Lambda_re, B_Lambda_im, B_B_re, B_B_im,
         B_C_re, B_C_im, B_log_dt, B_Dskip, gate_w):
    vec = pl.BlockSpec(memory_space=pltpu.VMEM)
    hbm = pl.BlockSpec(memory_space=pltpu.HBM)
    xt = jnp.transpose(A_x[0])
    wot = jnp.transpose(A_w_o, (0, 2, 1))
    out = pl.pallas_call(
        _kernel,
        in_specs=[hbm, hbm, hbm, hbm, hbm, hbm, vec, vec, hbm, hbm, hbm, hbm, vec, vec, vec],
        out_specs=hbm,
        out_shape=jax.ShapeDtypeStruct((M, S), F32),
        scratch_shapes=[
            pltpu.VMEM((M, S), BF16),
            pltpu.VMEM((S, DC), BF16),
            pltpu.VMEM((2, M, D), jnp.uint32),
            pltpu.VMEM((2, DC, D), jnp.uint32),
            pltpu.VMEM((2, DC, D), jnp.uint32),
            pltpu.VMEM((H, M, D), BF16),
            pltpu.VMEM((4, M, M), BF16),
            pltpu.VMEM((D, S), BF16),
            pltpu.VMEM((S, D), BF16),
            pltpu.VMEM((D, S), BF16),
            pltpu.VMEM((1, S), F32),
            pltpu.VMEM((H, D, S), BF16),
            pltpu.VMEM((M, S), F32),
            pltpu.VMEM((DC, D), BF16),
            pltpu.VMEM((M, 2 * M), BF16),
            pltpu.VMEM((2, S, M), F32),
            pltpu.VMEM((8, 8, M), F32),
            pltpu.SemaphoreType.DMA((2, 3)),
            pltpu.SemaphoreType.DMA((8,)),
            pltpu.SemaphoreType.DMA((S // OB,)),
        ],
        compiler_params=pltpu.CompilerParams(vmem_limit_bytes=100 * 2**20),
    )(xt, A_c_kv[0], A_w_q, A_w_uk, A_w_uv, wot, B_Lambda_re, B_Lambda_im, B_B_re, B_B_im,
      B_C_re, B_C_im, B_log_dt, B_Dskip, gate_w)
    return jnp.transpose(out)[None]
```
